```python
import os as _os
_os.environ.setdefault('JAX_PLATFORMS', 'cpu')
import jax
import jax.numpy as jnp

def _softmax(x, axis=-1):
    return jax.nn.softmax(x, axis=axis)

def _gelu(x):
    return jax.nn.gelu(x, approximate=True)

def _silu(x):
    return jax.nn.silu(x)

def _sigmoid(x):
    return jax.nn.sigmoid(x)

def _layernorm(x, axis=-1, eps=1e-05):
    m = jnp.mean(x, axis=axis, keepdims=True)
    v = jnp.var(x, axis=axis, keepdims=True)
    return (x - m) / jnp.sqrt(v + eps)

def _scatter_add(tgt, idx, src, axis=0):
    return tgt.at[idx].add(src)

def _segment_sum(src, seg, n):
    return jax.ops.segment_sum(src, seg, n)

class _Rng:

    def __init__(self, key):
        self._k = key

    def _next(self):
        self._k, sub = jax.random.split(self._k)
        return sub

    def normal(self, shape):
        return jax.random.normal(self._next(), shape, dtype=jnp.bfloat16)

    def randint(self, lo, hi, shape):
        return jax.random.randint(self._next(), shape, lo, hi, dtype=jnp.int32)

    def uniform(self, shape, lo=0.0, hi=1.0):
        return jax.random.uniform(self._next(), shape, jnp.bfloat16, lo, hi)

    def permutation(self, n):
        return jax.random.permutation(self._next(), n)
kernel_name = 'parallel_sum__memory_aug_recurrent_mem_tr__dense_activation_silu__prompt'

def setup_inputs():
    _rng = _Rng(jax.random.key(int.from_bytes(__import__("os").urandom(4), "little")))
    _w = lambda a: (lambda t: t.astype(jnp.bfloat16) if jnp.issubdtype(t.dtype, jnp.floating) else t)(jnp.asarray(a))

    def _A_setup():
        B, S, Dm = (1, 2048, 448)
        H, Dh = (16, 256)
        M, seg = (8, 32)
        seg = min(seg, S)
        S = S // seg * seg
        return {'x': _w((lambda *s: _rng.normal(s) * 0.05)(B, S, Dm)), 'mem0': _w((lambda *s: _rng.normal(s) * 0.2)(B, M, Dm)), 'Wq': _w((lambda *s: _rng.normal(s) * 0.8)(Dm, H, Dh) * Dm ** (-0.5)), 'Wk': _w((lambda *s: _rng.normal(s) * 0.8)(Dm, H, Dh) * Dm ** (-0.5)), 'Wv': _w((lambda *s: _rng.normal(s) * 0.2)(Dm, H, Dh) * Dm ** (-0.5)), 'Wo': _w((lambda *s: _rng.normal(s) * 0.2)(H, Dh, Dm) * (H * Dh) ** (-0.5)), 'seg_len': seg}
    _A_in = _A_setup()

    def _B_setup():
        B, S, D, F = (1, 2048, 448, 1792)
        return {'x': _w((lambda *s: _rng.normal(s) * 0.05)(B, S, D)), 'w1': _w((lambda *s: _rng.normal(s) * 0.05)(D, F) * D ** (-0.5)), 'w2': _w((lambda *s: _rng.normal(s) * 0.05)(F, D) * F ** (-0.5))}
    _B_in = _B_setup()
    return {'A_x': _A_in['x'], 'A_mem0': _A_in['mem0'], 'A_Wq': _A_in['Wq'], 'A_Wk': _A_in['Wk'], 'A_Wv': _A_in['Wv'], 'A_Wo': _A_in['Wo'], 'A_seg_len': _A_in['seg_len'], 'B_x': _B_in['x'], 'B_w1': _B_in['w1'], 'B_w2': _B_in['w2']}

def reference(A_x, A_mem0, A_Wq, A_Wk, A_Wv, A_Wo, A_seg_len, B_x, B_w1, B_w2):

    def _A_ref(x, mem0, Wq, Wk, Wv, Wo, seg_len):
        B, S, Dm = x.shape
        H, Dh = (Wq.shape[1], Wq.shape[2])
        M = mem0.shape[1]
        scale = Dh ** (-0.5)
        n_seg = S // seg_len
        L = M + seg_len
        idx = jnp.arange(L)
        mask = (idx[:, None] < M) | (idx[:, None] >= idx[None, :])
        mem = mem0
        outs = []
        for s in range(n_seg):
            xs = x[:, s * seg_len:(s + 1) * seg_len, :].copy()
            h = jnp.concatenate([mem, xs], axis=1)
            q = jnp.einsum('btd,dhe->bhte', h, Wq)
            k = jnp.einsum('btd,dhe->bhte', h, Wk)
            v = jnp.einsum('btd,dhe->bhte', h, Wv)
            scores = jnp.einsum('bhqe,bhke->bhqk', q, k) * scale
            scores = jnp.where(mask[None, None], scores, -1000000000.0)
            p = _softmax(scores, axis=-1)
            o = jnp.einsum('bhqk,bhke->bhqe', p, v)
            o = jnp.einsum('bhte,hed->btd', o, Wo)
            mem = o[:, :M, :].copy()
            outs.append(o[:, M:, :])
        return jnp.concatenate(outs, axis=1)

    def _B_ref(x, w1, w2):
        h = jnp.einsum('bsd,df->bsf', x, w1)
        h = _silu(h)
        out = jnp.einsum('bsf,fd->bsd', h, w2)
        return out
    x = A_x
    xn = _layernorm(x, axis=-1)
    return x + _A_ref(xn, A_mem0, A_Wq, A_Wk, A_Wv, A_Wo, A_seg_len) + _B_ref(xn, B_w1, B_w2)
```

```python
import functools

import jax
import jax.numpy as jnp
import numpy as np
import jax.experimental.pallas as pl
import jax.experimental.pallas.tpu as pltpu


_LN_EPS = 1e-05
_NEG = -1000000000.0


def _kernel(x_ref, mem0_ref, wqkv_ref, wo_ref, w1_ref, w2_ref, out_ref,
            mem_sc, qkv_sc, qall_sc, kall_sc, vall_sc, omem_sc, oxs_sc,
            *, seg, nseg, M, MP, KP, H, Dh):
    f32 = jnp.float32
    bf16 = jnp.bfloat16
    HD = H * Dh
    scale = float(Dh) ** (-0.5)

    @pl.when(pl.program_id(0) == 0)
    def _():
        m0 = mem0_ref[...].astype(f32)
        mem_sc[0:M, :] = m0
        mem_sc[M:MP, :] = jnp.zeros((MP - M, m0.shape[1]), f32)

    kall_sc[MP + seg:KP, :] = jnp.zeros((KP - MP - seg, HD), bf16)
    vall_sc[MP + seg:KP, :] = jnp.zeros((KP - MP - seg, HD), bf16)

    xf = x_ref[...].astype(f32)
    mu = jnp.mean(xf, axis=-1, keepdims=True)
    xc = xf - mu
    var = jnp.mean(xc * xc, axis=-1, keepdims=True)
    xn = xc / jnp.sqrt(var + _LN_EPS)
    xn_bf = xn.astype(bf16)

    NC = 1536
    for c in range(0, 3 * HD, NC):
        qkv_sc[:, c:c + NC] = jnp.dot(
            xn_bf, wqkv_ref[:, c:c + NC], preferred_element_type=f32).astype(bf16)

    QL = MP + seg
    qi = jax.lax.broadcasted_iota(jnp.int32, (QL, KP), 0)
    jj = jax.lax.broadcasted_iota(jnp.int32, (QL, KP), 1)
    valid = (jj < M) | ((jj >= MP) & (jj < QL) & ((qi < MP) | (jj <= qi)))

    def seg_body(j, carry):
        r0 = pl.multiple_of(j * seg, seg)
        mem_bf = mem_sc[...].astype(bf16)
        pm = jnp.dot(mem_bf, wqkv_ref[...], preferred_element_type=f32).astype(bf16)
        qall_sc[0:MP, :] = pm[:, 0:HD]
        kall_sc[0:MP, :] = pm[:, HD:2 * HD]
        vall_sc[0:MP, :] = pm[:, 2 * HD:3 * HD]
        qall_sc[MP:QL, :] = qkv_sc[pl.ds(r0, seg), 0:HD]
        kall_sc[MP:QL, :] = qkv_sc[pl.ds(r0, seg), HD:2 * HD]
        vall_sc[MP:QL, :] = qkv_sc[pl.ds(r0, seg), 2 * HD:3 * HD]
        for h in range(H):
            c0 = h * Dh
            q = qall_sc[:, c0:c0 + Dh]
            k = kall_sc[:, c0:c0 + Dh]
            v = vall_sc[:, c0:c0 + Dh]
            s = jax.lax.dot_general(q, k, (((1,), (1,)), ((), ())),
                                    preferred_element_type=f32)
            s = s * scale
            s = jnp.where(valid, s, _NEG)
            mx = jnp.max(s, axis=-1, keepdims=True)
            e = jnp.exp(s - mx)
            p = e / jnp.sum(e, axis=-1, keepdims=True)
            o = jnp.dot(p.astype(bf16), v, preferred_element_type=f32).astype(bf16)
            omem_sc[:, c0:c0 + Dh] = o[0:MP]
            oxs_sc[pl.ds(r0, seg), c0:c0 + Dh] = o[MP:QL]
        mem_new = jnp.dot(omem_sc[...], wo_ref[...], preferred_element_type=f32)
        mem_sc[0:M, :] = mem_new[0:M].astype(bf16).astype(f32)
        return carry

    jax.lax.fori_loop(0, nseg, seg_body, 0)

    outA = jnp.dot(oxs_sc[...], wo_ref[...], preferred_element_type=f32)
    hb = jnp.dot(xn_bf, w1_ref[...], preferred_element_type=f32)
    hb = hb * jax.nn.sigmoid(hb)
    outB = jnp.dot(hb.astype(bf16), w2_ref[...], preferred_element_type=f32)
    out_ref[...] = (xf + outA + outB).astype(out_ref.dtype)


@jax.jit
def pallas_parallel_sum__memory_aug_recurrent_mem_tr__dense_activation_silu__prompt_kernel(
    A_x: jax.Array,
    A_mem0: jax.Array,
    A_Wq: jax.Array,
    A_Wk: jax.Array,
    A_Wv: jax.Array,
    A_Wo: jax.Array,
    A_seg_len,
    B_x: jax.Array,
    B_w1: jax.Array,
    B_w2: jax.Array,
):
    B, S, D = A_x.shape
    assert B == 1
    H, Dh = A_Wq.shape[1], A_Wq.shape[2]
    M = A_mem0.shape[1]
    seg = int(A_seg_len) if isinstance(A_seg_len, (int, np.integer)) else 32
    assert S % seg == 0
    F = B_w1.shape[1]
    HD = H * Dh

    x = A_x.reshape(S, D)
    mem0 = A_mem0.reshape(M, D)
    wqkv = jnp.concatenate(
        [A_Wq.reshape(D, HD), A_Wk.reshape(D, HD), A_Wv.reshape(D, HD)], axis=1)
    wo = A_Wo.reshape(HD, D)
    w1 = B_w1
    w2 = B_w2

    BR = 256
    assert BR % seg == 0 and S % BR == 0
    nseg = BR // seg
    MP = 16
    KP = 128
    assert M <= MP and MP + seg <= KP

    kernel = functools.partial(_kernel, seg=seg, nseg=nseg, M=M, MP=MP, KP=KP, H=H, Dh=Dh)

    grid = (S // BR,)
    in_specs = [
        pl.BlockSpec((BR, D), lambda i: (i, 0)),
        pl.BlockSpec((M, D), lambda i: (0, 0)),
        pl.BlockSpec((D, 3 * HD), lambda i: (0, 0)),
        pl.BlockSpec((HD, D), lambda i: (0, 0)),
        pl.BlockSpec((D, F), lambda i: (0, 0)),
        pl.BlockSpec((F, D), lambda i: (0, 0)),
    ]
    out_specs = pl.BlockSpec((BR, D), lambda i: (i, 0))
    scratch_shapes = [
        pltpu.VMEM((MP, D), jnp.float32),
        pltpu.VMEM((BR, 3 * HD), jnp.bfloat16),
        pltpu.VMEM((MP + seg, HD), jnp.bfloat16),
        pltpu.VMEM((KP, HD), jnp.bfloat16),
        pltpu.VMEM((KP, HD), jnp.bfloat16),
        pltpu.VMEM((MP, HD), jnp.bfloat16),
        pltpu.VMEM((BR, HD), jnp.bfloat16),
    ]
    out = pl.pallas_call(
        kernel,
        grid=grid,
        in_specs=in_specs,
        out_specs=out_specs,
        out_shape=jax.ShapeDtypeStruct((S, D), A_x.dtype),
        scratch_shapes=scratch_shapes,
        compiler_params=pltpu.CompilerParams(
            dimension_semantics=("arbitrary",),
            vmem_limit_bytes=110 * 1024 * 1024,
        ),
    )(x, mem0, wqkv, wo, w1, w2)
    return out.reshape(B, S, D)
```

```python
import functools

import jax
import jax.numpy as jnp
import numpy as np
import jax.experimental.pallas as pl
import jax.experimental.pallas.tpu as pltpu


_LN_EPS = 1e-05
_NEG = -1000000000.0


def _kernel(x_ref, mem0_ref, wq_ref, wk_ref, wv_ref, wo_in_ref, w1_in_ref, w2_in_ref, out_ref,
            mem_sc, qall_sc, kall_sc, vall_sc, o_sc, s_sc, p_sc,
            wqkv_ref, wo_ref, w1_ref, w2_ref,
            *, seg, npair, M, QL, KP, H, Dh):
    f32 = jnp.float32
    bf16 = jnp.bfloat16
    u32 = jnp.uint32
    HD = H * Dh
    scale = float(Dh) ** (-0.5)
    assert QL == seg + 2 * M and M % 8 == 0

    @pl.when(pl.program_id(0) == 0)
    def _():
        mem_sc[...] = mem0_ref[...].astype(f32)
        wqkv_ref[:, 0:HD] = pltpu.bitcast(wq_ref[...], u32)
        wqkv_ref[:, HD:2 * HD] = pltpu.bitcast(wk_ref[...], u32)
        wqkv_ref[:, 2 * HD:3 * HD] = pltpu.bitcast(wv_ref[...], u32)
        wo_ref[...] = pltpu.bitcast(wo_in_ref[...], u32)
        w1_ref[...] = pltpu.bitcast(w1_in_ref[...], u32)
        w2_ref[...] = pltpu.bitcast(w2_in_ref[...], u32)

    kall_sc[QL:KP, :] = jnp.zeros((KP - QL, HD), bf16)
    vall_sc[QL:KP, :] = jnp.zeros((KP - QL, HD), bf16)

    qi = jax.lax.broadcasted_iota(jnp.int32, (QL, KP), 0)
    jj = jax.lax.broadcasted_iota(jnp.int32, (QL, KP), 1)
    valid = (jj < M) | ((jj < M + seg) & ((qi < M) | (jj <= qi)))

    NC = 2048
    bufs = (qall_sc, kall_sc, vall_sc)

    def ffn(xn_bf):
        hb = jnp.dot(xn_bf, pltpu.bitcast(w1_ref[...], bf16),
                     preferred_element_type=f32)
        hb = hb * jax.nn.sigmoid(hb)
        outB = jnp.dot(hb.astype(bf16), pltpu.bitcast(w2_ref[...], bf16),
                       preferred_element_type=f32)
        return outB

    def attend_and_project(xn_bf):
        for h_ in range(H):
            c0 = h_ * Dh
            q = qall_sc[:, c0:c0 + Dh]
            k = kall_sc[:, c0:c0 + Dh]
            s = jax.lax.dot_general(q, k, (((1,), (1,)), ((), ())),
                                    preferred_element_type=f32)
            s_sc[h_ * QL:(h_ + 1) * QL, :] = jnp.where(valid, s * scale, _NEG)
        outB = ffn(xn_bf)
        sall = s_sc[...]
        mx = jnp.max(sall, axis=-1, keepdims=True)
        e = jnp.exp(sall - mx)
        p = e * pl.reciprocal(jnp.sum(e, axis=-1, keepdims=True), approx=False)
        p_sc[...] = p.astype(bf16)
        for h_ in range(H):
            c0 = h_ * Dh
            ph = p_sc[h_ * QL:(h_ + 1) * QL, :]
            v = vall_sc[:, c0:c0 + Dh]
            o_sc[:, c0:c0 + Dh] = jnp.dot(
                ph, v, preferred_element_type=f32).astype(bf16)
        res = jnp.dot(o_sc[...], pltpu.bitcast(wo_ref[...], bf16),
                      preferred_element_type=f32)
        mem_sc[...] = res[0:M].astype(bf16).astype(f32)
        return res, outB

    def pair_body(t, carry):
        r0 = pl.multiple_of(t * (2 * seg), 2 * seg)
        xf = x_ref[pl.ds(r0, 2 * seg), :].astype(f32)
        mu = jnp.mean(xf, axis=-1, keepdims=True)
        xc = xf - mu
        var = jnp.mean(xc * xc, axis=-1, keepdims=True)
        xn = xc / jnp.sqrt(var + _LN_EPS)
        xn_bf = xn.astype(bf16)

        h = jnp.concatenate([mem_sc[...], xn[0:seg + M]], axis=0).astype(bf16)
        for c in range(0, 3 * HD, NC):
            r = jnp.dot(h, pltpu.bitcast(wqkv_ref[:, c:c + NC], bf16),
                        preferred_element_type=f32)
            bufs[c // HD][0:QL, (c % HD):(c % HD) + NC] = r.astype(bf16)
        res, outB = attend_and_project(xn_bf[0:seg])
        out_ref[pl.ds(r0, seg), :] = (
            xf[0:seg] + res[M:M + seg] + outB).astype(out_ref.dtype)

        for b in bufs:
            b[M:2 * M, :] = b[M + seg:QL, :]
        h = jnp.concatenate([mem_sc[...], xn[seg + M:2 * seg]], axis=0).astype(bf16)
        for c in range(0, 3 * HD, NC):
            r = jnp.dot(h, pltpu.bitcast(wqkv_ref[:, c:c + NC], bf16),
                        preferred_element_type=f32)
            b = bufs[c // HD]
            b[0:M, (c % HD):(c % HD) + NC] = r[0:M].astype(bf16)
            b[2 * M:M + seg, (c % HD):(c % HD) + NC] = r[M:seg].astype(bf16)
        res, outB = attend_and_project(xn_bf[seg:2 * seg])
        out_ref[pl.ds(pl.multiple_of(r0 + seg, seg), seg), :] = (
            xf[seg:2 * seg] + res[M:M + seg] + outB).astype(out_ref.dtype)
        return carry

    jax.lax.fori_loop(0, npair, pair_body, 0)


@jax.jit
def pallas_parallel_sum__memory_aug_recurrent_mem_tr__dense_activation_silu__prompt_kernel(
    A_x: jax.Array,
    A_mem0: jax.Array,
    A_Wq: jax.Array,
    A_Wk: jax.Array,
    A_Wv: jax.Array,
    A_Wo: jax.Array,
    A_seg_len,
    B_x: jax.Array,
    B_w1: jax.Array,
    B_w2: jax.Array,
):
    B, S, D = A_x.shape
    assert B == 1
    H, Dh = A_Wq.shape[1], A_Wq.shape[2]
    M = A_mem0.shape[1]
    seg = int(A_seg_len) if isinstance(A_seg_len, (int, np.integer)) else 32
    assert S % seg == 0
    F = B_w1.shape[1]
    HD = H * Dh

    x = A_x.reshape(S, D)
    mem0 = A_mem0.reshape(M, D)
    wq = A_Wq.reshape(D, HD)
    wk = A_Wk.reshape(D, HD)
    wv = A_Wv.reshape(D, HD)
    wo = A_Wo.reshape(HD, D)
    w1 = B_w1
    w2 = B_w2

    BR = 256
    assert BR % (2 * seg) == 0 and S % BR == 0
    npair = BR // (2 * seg)
    QL = seg + 2 * M
    KP = 128
    assert QL <= KP and M % 8 == 0 and QL % 16 == 0

    kernel = functools.partial(_kernel, seg=seg, npair=npair, M=M, QL=QL, KP=KP, H=H, Dh=Dh)

    grid = (S // BR,)
    in_specs = [
        pl.BlockSpec((BR, D), lambda i: (i, 0)),
        pl.BlockSpec((M, D), lambda i: (0, 0)),
        pl.BlockSpec((D, HD), lambda i: (0, 0), pipeline_mode=pl.Buffered(1)),
        pl.BlockSpec((D, HD), lambda i: (0, 0), pipeline_mode=pl.Buffered(1)),
        pl.BlockSpec((D, HD), lambda i: (0, 0), pipeline_mode=pl.Buffered(1)),
        pl.BlockSpec((HD, D), lambda i: (0, 0), pipeline_mode=pl.Buffered(1)),
        pl.BlockSpec((D, F), lambda i: (0, 0), pipeline_mode=pl.Buffered(1)),
        pl.BlockSpec((F, D), lambda i: (0, 0), pipeline_mode=pl.Buffered(1)),
    ]
    out_specs = pl.BlockSpec((BR, D), lambda i: (i, 0))
    scratch_shapes = [
        pltpu.VMEM((M, D), jnp.float32),
        pltpu.VMEM((QL, HD), jnp.bfloat16),
        pltpu.VMEM((KP, HD), jnp.bfloat16),
        pltpu.VMEM((KP, HD), jnp.bfloat16),
        pltpu.VMEM((QL, HD), jnp.bfloat16),
        pltpu.VMEM((H * QL, KP), jnp.float32),
        pltpu.VMEM((H * QL, KP), jnp.bfloat16),
        pltpu.VMEM((D // 2, 3 * HD), jnp.uint32),
        pltpu.VMEM((HD // 2, D), jnp.uint32),
        pltpu.VMEM((D // 2, F), jnp.uint32),
        pltpu.VMEM((F // 2, D), jnp.uint32),
    ]
    out = pl.pallas_call(
        kernel,
        grid=grid,
        in_specs=in_specs,
        out_specs=out_specs,
        out_shape=jax.ShapeDtypeStruct((S, D), A_x.dtype),
        scratch_shapes=scratch_shapes,
        compiler_params=pltpu.CompilerParams(
            dimension_semantics=("arbitrary",),
            vmem_limit_bytes=110 * 1024 * 1024,
        ),
    )(x, mem0, wq, wk, wv, wo, w1, w2)
    return out.reshape(B, S, D)
```

```python
import functools

import jax
import jax.numpy as jnp
import numpy as np
import jax.experimental.pallas as pl
import jax.experimental.pallas.tpu as pltpu


_LN_EPS = 1e-05
_NEG = -1000000000.0


def _kernel(xT_ref, mem0_ref, wq_hbm, wk_hbm, wv_hbm, woT_hbm, w1_hbm, w2T_hbm, outT_ref,
            mem_sc, x_ref, out_ref, qall_sc, kall_sc, vall_sc, o_sc, s_sc, p_sc,
            wqkv_ref, wo_ref, w1_ref, w2_ref,
            raw_q, raw_k, raw_v, raw_o, raw_1, raw_2, dsem,
            *, seg, npair, M, QL, KP, H, Dh):
    f32 = jnp.float32
    bf16 = jnp.bfloat16
    u32 = jnp.uint32
    HD = H * Dh
    scale = float(Dh) ** (-0.5)
    assert QL == seg + 2 * M and M % 8 == 0

    @pl.when(pl.program_id(0) == 0)
    def _():
        srcs = (wq_hbm, wk_hbm, wv_hbm, woT_hbm, w1_hbm, w2T_hbm)
        dsts = (raw_q, raw_k, raw_v, raw_o, raw_1, raw_2)
        cps = [pltpu.make_async_copy(srcs[i], dsts[i], dsem.at[i]) for i in range(6)]
        cps[0].start()
        cps[1].start()
        mem_sc[...] = mem0_ref[...].astype(f32)
        D_ = raw_q.shape[0]

        def relayout(w_in, w_i):
            def grp(g, carry):
                v = w_in[pl.ds(pl.multiple_of(g * 16, 16), 16)].reshape(16, HD)
                wqkv_ref[pl.ds(pl.multiple_of(g * 8, 8), 8),
                         w_i * HD:(w_i + 1) * HD] = pltpu.bitcast(v, u32)
                return carry
            jax.lax.fori_loop(0, D_ // 16, grp, 0)

        cps[0].wait()
        cps[2].start()
        relayout(raw_q, 0)
        cps[1].wait()
        cps[4].start()
        relayout(raw_k, 1)
        cps[2].wait()
        cps[3].start()
        relayout(raw_v, 2)
        cps[4].wait()
        cps[5].start()
        w1_ref[...] = pltpu.bitcast(raw_1[...], u32)
        cps[3].wait()
        for h_ in range(H):
            wo_ref[h_ * Dh // 2:(h_ + 1) * Dh // 2, :] = pltpu.bitcast(
                raw_o[h_].astype(f32).T.astype(bf16), u32)
        cps[5].wait()
        F = raw_2.shape[1]
        for c in range(0, F, Dh):
            w2_ref[c // 2:(c + Dh) // 2, :] = pltpu.bitcast(
                raw_2[:, c:c + Dh].astype(f32).T.astype(bf16), u32)

    kall_sc[QL:KP, :] = jnp.zeros((KP - QL, HD), bf16)
    vall_sc[QL:KP, :] = jnp.zeros((KP - QL, HD), bf16)

    qi = jax.lax.broadcasted_iota(jnp.int32, (QL, KP), 0)
    jj = jax.lax.broadcasted_iota(jnp.int32, (QL, KP), 1)
    valid = (jj < M) | ((jj < M + seg) & ((qi < M) | (jj <= qi)))

    NC = 2048
    bufs = (qall_sc, kall_sc, vall_sc)

    def ffn1(xn_bf):
        hb = jnp.dot(xn_bf, pltpu.bitcast(w1_ref[...], bf16),
                     preferred_element_type=f32)
        hb = (hb * jax.nn.sigmoid(hb)).astype(bf16)
        return hb

    def ffn2(hb):
        outB = jnp.dot(hb, pltpu.bitcast(w2_ref[...], bf16),
                       preferred_element_type=f32)
        return outB

    def attend(xn_bf):
        hb = ffn1(xn_bf)
        for h_ in range(H):
            c0 = h_ * Dh
            q = qall_sc[:, c0:c0 + Dh]
            k = kall_sc[:, c0:c0 + Dh]
            s = jax.lax.dot_general(q, k, (((1,), (1,)), ((), ())),
                                    preferred_element_type=f32)
            s_sc[h_ * QL:(h_ + 1) * QL, :] = jnp.where(valid, s * scale, _NEG)
        sall = s_sc[...]
        mx = jnp.max(sall, axis=-1, keepdims=True)
        e = jnp.exp(sall - mx)
        p = e * pl.reciprocal(jnp.sum(e, axis=-1, keepdims=True), approx=False)
        p_sc[...] = p.astype(bf16)
        outB = ffn2(hb)
        for h_ in range(H):
            c0 = h_ * Dh
            ph = p_sc[h_ * QL:(h_ + 1) * QL, :]
            v = vall_sc[:, c0:c0 + Dh]
            o = jnp.dot(ph, v, preferred_element_type=f32)
            o_sc[0:M + seg, c0:c0 + Dh] = o[0:M + seg].astype(bf16)
        return outB

    def out_project(nrows):
        res = jnp.dot(o_sc[0:nrows, :], pltpu.bitcast(wo_ref[...], bf16),
                      preferred_element_type=f32)
        mem_sc[...] = res[0:M].astype(bf16).astype(f32)
        return res

    x_ref[...] = xT_ref[...].astype(f32).T

    def pair_body(t, carry):
        r0 = pl.multiple_of(t * (2 * seg), 2 * seg)
        xf = x_ref[pl.ds(r0, 2 * seg), :]
        mu = jnp.mean(xf, axis=-1, keepdims=True)
        xc = xf - mu
        var = jnp.mean(xc * xc, axis=-1, keepdims=True)
        xn = xc / jnp.sqrt(var + _LN_EPS)
        xn_bf = xn.astype(bf16)

        h = jnp.concatenate([mem_sc[...], xn[0:seg + M]], axis=0).astype(bf16)
        for c in range(0, 3 * HD, NC):
            r = jnp.dot(h, pltpu.bitcast(wqkv_ref[:, c:c + NC], bf16),
                        preferred_element_type=f32)
            bufs[c // HD][0:QL, (c % HD):(c % HD) + NC] = r.astype(bf16)
        outB = attend(xn_bf[0:seg])
        res = out_project(seg)
        out_ref[pl.ds(r0, seg), :] = xf[0:seg] + outB + jnp.concatenate(
            [res[M:seg], jnp.zeros((M, res.shape[1]), f32)], axis=0)
        o_sc[M + seg:QL, :] = o_sc[seg:M + seg, :]

        for b in bufs:
            b[M:2 * M, :] = b[M + seg:QL, :]
        h = jnp.concatenate([mem_sc[...], xn[seg + M:2 * seg]], axis=0).astype(bf16)
        for c in range(0, 3 * HD, NC):
            r = jnp.dot(h, pltpu.bitcast(wqkv_ref[:, c:c + NC], bf16),
                        preferred_element_type=f32)
            b = bufs[c // HD]
            b[0:M, (c % HD):(c % HD) + NC] = r[0:M].astype(bf16)
            b[2 * M:M + seg, (c % HD):(c % HD) + NC] = r[M:seg].astype(bf16)
        outB = attend(xn_bf[seg:2 * seg])
        res = out_project(QL)
        out_ref[pl.ds(pl.multiple_of(r0 + seg, seg), seg), :] = (
            xf[seg:2 * seg] + res[M:M + seg] + outB)
        rl = pl.multiple_of(r0 + seg - M, M)
        out_ref[pl.ds(rl, M), :] = out_ref[pl.ds(rl, M), :] + res[M + seg:QL]
        return carry

    jax.lax.fori_loop(0, npair, pair_body, 0)
    outT_ref[...] = out_ref[...].T.astype(outT_ref.dtype)


@jax.jit
def pallas_parallel_sum__memory_aug_recurrent_mem_tr__dense_activation_silu__prompt_kernel(
    A_x: jax.Array,
    A_mem0: jax.Array,
    A_Wq: jax.Array,
    A_Wk: jax.Array,
    A_Wv: jax.Array,
    A_Wo: jax.Array,
    A_seg_len,
    B_x: jax.Array,
    B_w1: jax.Array,
    B_w2: jax.Array,
):
    B, S, D = A_x.shape
    assert B == 1
    H, Dh = A_Wq.shape[1], A_Wq.shape[2]
    M = A_mem0.shape[1]
    seg = int(A_seg_len) if isinstance(A_seg_len, (int, np.integer)) else 32
    assert S % seg == 0
    F = B_w1.shape[1]
    HD = H * Dh

    xT = jnp.transpose(A_x, (0, 2, 1)).reshape(D, S)
    mem0 = A_mem0.reshape(M, D)
    wq, wk, wv = A_Wq, A_Wk, A_Wv
    woT = jnp.transpose(A_Wo, (0, 2, 1))
    w1 = B_w1
    w2T = B_w2.T

    BR = 256
    assert BR % (2 * seg) == 0 and S % BR == 0
    npair = BR // (2 * seg)
    QL = seg + 2 * M
    KP = 128
    assert QL <= KP and M % 8 == 0 and QL % 16 == 0

    kernel = functools.partial(_kernel, seg=seg, npair=npair, M=M, QL=QL, KP=KP, H=H, Dh=Dh)

    grid = (S // BR,)
    in_specs = [
        pl.BlockSpec((D, BR), lambda i: (0, i)),
        pl.BlockSpec((M, D), lambda i: (0, 0)),
        pl.BlockSpec(memory_space=pl.ANY),
        pl.BlockSpec(memory_space=pl.ANY),
        pl.BlockSpec(memory_space=pl.ANY),
        pl.BlockSpec(memory_space=pl.ANY),
        pl.BlockSpec(memory_space=pl.ANY),
        pl.BlockSpec(memory_space=pl.ANY),
    ]
    out_specs = pl.BlockSpec((D, BR), lambda i: (0, i))
    scratch_shapes = [
        pltpu.VMEM((M, D), jnp.float32),
        pltpu.VMEM((BR, D), jnp.float32),
        pltpu.VMEM((BR, D), jnp.float32),
        pltpu.VMEM((QL, HD), jnp.bfloat16),
        pltpu.VMEM((KP, HD), jnp.bfloat16),
        pltpu.VMEM((KP, HD), jnp.bfloat16),
        pltpu.VMEM((QL, HD), jnp.bfloat16),
        pltpu.VMEM((H * QL, KP), jnp.float32),
        pltpu.VMEM((H * QL, KP), jnp.bfloat16),
        pltpu.VMEM((D // 2, 3 * HD), jnp.uint32),
        pltpu.VMEM((HD // 2, D), jnp.uint32),
        pltpu.VMEM((D // 2, F), jnp.uint32),
        pltpu.VMEM((F // 2, D), jnp.uint32),
        pltpu.VMEM((D, H, Dh), jnp.bfloat16),
        pltpu.VMEM((D, H, Dh), jnp.bfloat16),
        pltpu.VMEM((D, H, Dh), jnp.bfloat16),
        pltpu.VMEM((H, D, Dh), jnp.bfloat16),
        pltpu.VMEM((D, F), jnp.bfloat16),
        pltpu.VMEM((D, F), jnp.bfloat16),
        pltpu.SemaphoreType.DMA((6,)),
    ]
    out = pl.pallas_call(
        kernel,
        grid=grid,
        in_specs=in_specs,
        out_specs=out_specs,
        out_shape=jax.ShapeDtypeStruct((D, S), A_x.dtype),
        scratch_shapes=scratch_shapes,
        compiler_params=pltpu.CompilerParams(
            dimension_semantics=("arbitrary",),
            vmem_limit_bytes=110 * 1024 * 1024,
        ),
    )(xT, mem0, wq, wk, wv, woT, w1, w2T)
    return jnp.transpose(out.reshape(B, D, S), (0, 2, 1))
```

```python
import functools

import jax
import jax.numpy as jnp
import numpy as np
import jax.experimental.pallas as pl
import jax.experimental.pallas.tpu as pltpu


_LN_EPS = 1e-05
_NEG = -1000000000.0


def _kernel(xT_ref, mem0_ref, wq_hbm, wk_hbm, wv_hbm, woT_hbm, w1_hbm, w2T_hbm, outT_ref,
            mem_sc, x_ref, out_ref, qall_sc, kall_sc, vall_sc, o_sc, s_sc, p_sc,
            wqkv_ref, wo_ref, w1_ref, w2_ref,
            raw_q, raw_k, raw_v, raw_o, raw_1, raw_2, dsem,
            *, seg, npair, M, QL, KP, H, Dh):
    f32 = jnp.float32
    bf16 = jnp.bfloat16
    u32 = jnp.uint32
    HD = H * Dh
    scale = float(Dh) ** (-0.5)
    assert QL == seg + 2 * M and M % 8 == 0

    @pl.when(pl.program_id(0) == 0)
    def _():
        srcs = (wq_hbm, wk_hbm, wv_hbm, woT_hbm, w1_hbm, w2T_hbm)
        dsts = (raw_q, raw_k, raw_v, raw_o, raw_1, raw_2)
        cps = [pltpu.make_async_copy(srcs[i], dsts[i], dsem.at[i]) for i in range(6)]
        cps[0].start()
        cps[1].start()
        mem_sc[...] = mem0_ref[...].astype(f32)
        D_ = raw_q.shape[0]

        def relayout(w_in, w_i):
            def grp(g, carry):
                v = w_in[pl.ds(pl.multiple_of(g * 16, 16), 16)].reshape(16, HD)
                wqkv_ref[pl.ds(pl.multiple_of(g * 8, 8), 8),
                         w_i * HD:(w_i + 1) * HD] = pltpu.bitcast(v, u32)
                return carry
            jax.lax.fori_loop(0, D_ // 16, grp, 0)

        cps[0].wait()
        cps[2].start()
        relayout(raw_q, 0)
        cps[1].wait()
        cps[4].start()
        relayout(raw_k, 1)
        cps[2].wait()
        cps[3].start()
        relayout(raw_v, 2)
        cps[4].wait()
        cps[5].start()
        w1_ref[...] = pltpu.bitcast(raw_1[...], u32)
        cps[3].wait()
        for h_ in range(H):
            wo_ref[h_ * Dh // 2:(h_ + 1) * Dh // 2, :] = pltpu.bitcast(
                raw_o[h_].astype(f32).T.astype(bf16), u32)
        cps[5].wait()
        F = raw_2.shape[1]
        for c in range(0, F, Dh):
            w2_ref[c // 2:(c + Dh) // 2, :] = pltpu.bitcast(
                raw_2[:, c:c + Dh].astype(f32).T.astype(bf16), u32)

    kall_sc[QL:KP, :] = jnp.zeros((KP - QL, HD), bf16)
    vall_sc[QL:KP, :] = jnp.zeros((KP - QL, HD), bf16)

    qi = jax.lax.broadcasted_iota(jnp.int32, (QL, KP), 0)
    jj = jax.lax.broadcasted_iota(jnp.int32, (QL, KP), 1)
    valid = (jj < M) | ((jj < M + seg) & ((qi < M) | (jj <= qi)))

    NC = 2048
    bufs = (qall_sc, kall_sc, vall_sc)

    def ffn1(xn_bf):
        hb = jnp.dot(xn_bf, pltpu.bitcast(w1_ref[...], bf16),
                     preferred_element_type=f32)
        hb = (hb * jax.nn.sigmoid(hb)).astype(bf16)
        return hb

    def ffn2(hb):
        outB = jnp.dot(hb, pltpu.bitcast(w2_ref[...], bf16),
                       preferred_element_type=f32)
        return outB

    def attend(xn_bf, v_proj):
        for h_ in range(H):
            c0 = h_ * Dh
            q = qall_sc[:, c0:c0 + Dh]
            k = kall_sc[:, c0:c0 + Dh]
            s = jax.lax.dot_general(q, k, (((1,), (1,)), ((), ())),
                                    preferred_element_type=f32)
            s_sc[h_ * QL:(h_ + 1) * QL, :] = jnp.where(valid, s * scale, _NEG)
        v_proj()
        hb = ffn1(xn_bf)
        sall = s_sc[...]
        mx = jnp.max(sall, axis=-1, keepdims=True)
        e = jnp.exp(sall - mx)
        p = e * pl.reciprocal(jnp.sum(e, axis=-1, keepdims=True), approx=False)
        p_sc[...] = p.astype(bf16)
        outB = ffn2(hb)
        for h_ in range(H):
            c0 = h_ * Dh
            ph = p_sc[h_ * QL:(h_ + 1) * QL, :]
            v = vall_sc[:, c0:c0 + Dh]
            o = jnp.dot(ph, v, preferred_element_type=f32)
            o_sc[0:M + seg, c0:c0 + Dh] = o[0:M + seg].astype(bf16)
        return outB

    def out_project(nrows):
        res = jnp.dot(o_sc[0:nrows, :], pltpu.bitcast(wo_ref[...], bf16),
                      preferred_element_type=f32)
        mem_sc[...] = res[0:M].astype(bf16).astype(f32)
        return res

    x_ref[...] = xT_ref[...].astype(f32).T

    def pair_body(t, carry):
        r0 = pl.multiple_of(t * (2 * seg), 2 * seg)
        xf = x_ref[pl.ds(r0, 2 * seg), :]
        mu = jnp.mean(xf, axis=-1, keepdims=True)
        xc = xf - mu
        var = jnp.mean(xc * xc, axis=-1, keepdims=True)
        xn = xc / jnp.sqrt(var + _LN_EPS)
        xn_bf = xn.astype(bf16)

        h = jnp.concatenate([mem_sc[...], xn[0:seg + M]], axis=0).astype(bf16)
        def proj_even(cs, h=h):
            for c in cs:
                r = jnp.dot(h, pltpu.bitcast(wqkv_ref[:, c:c + NC], bf16),
                            preferred_element_type=f32)
                bufs[c // HD][0:QL, (c % HD):(c % HD) + NC] = r.astype(bf16)
        proj_even(range(0, 2 * HD, NC))
        outB = attend(xn_bf[0:seg], lambda: proj_even(range(2 * HD, 3 * HD, NC)))
        res = out_project(seg)
        out_ref[pl.ds(r0, seg), :] = xf[0:seg] + outB + jnp.concatenate(
            [res[M:seg], jnp.zeros((M, res.shape[1]), f32)], axis=0)
        o_sc[M + seg:QL, :] = o_sc[seg:M + seg, :]

        for b in bufs:
            b[M:2 * M, :] = b[M + seg:QL, :]
        h = jnp.concatenate([mem_sc[...], xn[seg + M:2 * seg]], axis=0).astype(bf16)
        def proj_odd(cs, h=h):
            for c in cs:
                r = jnp.dot(h, pltpu.bitcast(wqkv_ref[:, c:c + NC], bf16),
                            preferred_element_type=f32)
                b = bufs[c // HD]
                b[0:M, (c % HD):(c % HD) + NC] = r[0:M].astype(bf16)
                b[2 * M:M + seg, (c % HD):(c % HD) + NC] = r[M:seg].astype(bf16)
        proj_odd(range(0, 2 * HD, NC))
        outB = attend(xn_bf[seg:2 * seg], lambda: proj_odd(range(2 * HD, 3 * HD, NC)))
        res = out_project(QL)
        out_ref[pl.ds(pl.multiple_of(r0 + seg, seg), seg), :] = (
            xf[seg:2 * seg] + res[M:M + seg] + outB)
        rl = pl.multiple_of(r0 + seg - M, M)
        out_ref[pl.ds(rl, M), :] = out_ref[pl.ds(rl, M), :] + res[M + seg:QL]
        return carry

    jax.lax.fori_loop(0, npair, pair_body, 0, unroll=True)
    outT_ref[...] = out_ref[...].T.astype(outT_ref.dtype)


@jax.jit
def pallas_parallel_sum__memory_aug_recurrent_mem_tr__dense_activation_silu__prompt_kernel(
    A_x: jax.Array,
    A_mem0: jax.Array,
    A_Wq: jax.Array,
    A_Wk: jax.Array,
    A_Wv: jax.Array,
    A_Wo: jax.Array,
    A_seg_len,
    B_x: jax.Array,
    B_w1: jax.Array,
    B_w2: jax.Array,
):
    B, S, D = A_x.shape
    assert B == 1
    H, Dh = A_Wq.shape[1], A_Wq.shape[2]
    M = A_mem0.shape[1]
    seg = int(A_seg_len) if isinstance(A_seg_len, (int, np.integer)) else 32
    assert S % seg == 0
    F = B_w1.shape[1]
    HD = H * Dh

    xT = jnp.transpose(A_x, (0, 2, 1)).reshape(D, S)
    mem0 = A_mem0.reshape(M, D)
    wq, wk, wv = A_Wq, A_Wk, A_Wv
    woT = jnp.transpose(A_Wo, (0, 2, 1))
    w1 = B_w1
    w2T = B_w2.T

    BR = 256
    assert BR % (2 * seg) == 0 and S % BR == 0
    npair = BR // (2 * seg)
    QL = seg + 2 * M
    KP = 128
    assert QL <= KP and M % 8 == 0 and QL % 16 == 0

    kernel = functools.partial(_kernel, seg=seg, npair=npair, M=M, QL=QL, KP=KP, H=H, Dh=Dh)

    grid = (S // BR,)
    in_specs = [
        pl.BlockSpec((D, BR), lambda i: (0, i)),
        pl.BlockSpec((M, D), lambda i: (0, 0)),
        pl.BlockSpec(memory_space=pl.ANY),
        pl.BlockSpec(memory_space=pl.ANY),
        pl.BlockSpec(memory_space=pl.ANY),
        pl.BlockSpec(memory_space=pl.ANY),
        pl.BlockSpec(memory_space=pl.ANY),
        pl.BlockSpec(memory_space=pl.ANY),
    ]
    out_specs = pl.BlockSpec((D, BR), lambda i: (0, i))
    scratch_shapes = [
        pltpu.VMEM((M, D), jnp.float32),
        pltpu.VMEM((BR, D), jnp.float32),
        pltpu.VMEM((BR, D), jnp.float32),
        pltpu.VMEM((QL, HD), jnp.bfloat16),
        pltpu.VMEM((KP, HD), jnp.bfloat16),
        pltpu.VMEM((KP, HD), jnp.bfloat16),
        pltpu.VMEM((QL, HD), jnp.bfloat16),
        pltpu.VMEM((H * QL, KP), jnp.float32),
        pltpu.VMEM((H * QL, KP), jnp.bfloat16),
        pltpu.VMEM((D // 2, 3 * HD), jnp.uint32),
        pltpu.VMEM((HD // 2, D), jnp.uint32),
        pltpu.VMEM((D // 2, F), jnp.uint32),
        pltpu.VMEM((F // 2, D), jnp.uint32),
        pltpu.VMEM((D, H, Dh), jnp.bfloat16),
        pltpu.VMEM((D, H, Dh), jnp.bfloat16),
        pltpu.VMEM((D, H, Dh), jnp.bfloat16),
        pltpu.VMEM((H, D, Dh), jnp.bfloat16),
        pltpu.VMEM((D, F), jnp.bfloat16),
        pltpu.VMEM((D, F), jnp.bfloat16),
        pltpu.SemaphoreType.DMA((6,)),
    ]
    out = pl.pallas_call(
        kernel,
        grid=grid,
        in_specs=in_specs,
        out_specs=out_specs,
        out_shape=jax.ShapeDtypeStruct((D, S), A_x.dtype),
        scratch_shapes=scratch_shapes,
        compiler_params=pltpu.CompilerParams(
            dimension_semantics=("arbitrary",),
            vmem_limit_bytes=110 * 1024 * 1024,
        ),
    )(xT, mem0, wq, wk, wv, woT, w1, w2T)
    return jnp.transpose(out.reshape(B, D, S), (0, 2, 1))
```
